```python
import os as _os
_os.environ.setdefault('JAX_PLATFORMS', 'cpu')
import jax
import jax.numpy as jnp

def _softmax(x, axis=-1):
    return jax.nn.softmax(x, axis=axis)

def _gelu(x):
    return jax.nn.gelu(x, approximate=True)

def _silu(x):
    return jax.nn.silu(x)

def _sigmoid(x):
    return jax.nn.sigmoid(x)

def _layernorm(x, axis=-1, eps=1e-05):
    m = jnp.mean(x, axis=axis, keepdims=True)
    v = jnp.var(x, axis=axis, keepdims=True)
    return (x - m) / jnp.sqrt(v + eps)

def _scatter_add(tgt, idx, src, axis=0):
    return tgt.at[idx].add(src)

def _segment_sum(src, seg, n):
    return jax.ops.segment_sum(src, seg, n)

class _Rng:

    def __init__(self, key):
        self._k = key

    def _next(self):
        self._k, sub = jax.random.split(self._k)
        return sub

    def normal(self, shape):
        return jax.random.normal(self._next(), shape, dtype=jnp.bfloat16)

    def randint(self, lo, hi, shape):
        return jax.random.randint(self._next(), shape, lo, hi, dtype=jnp.int32)

    def uniform(self, shape, lo=0.0, hi=1.0):
        return jax.random.uniform(self._next(), shape, jnp.bfloat16, lo, hi)

    def permutation(self, n):
        return jax.random.permutation(self._next(), n)
kernel_name = 'standalone__conformer_conv_module__speech'

def setup_inputs():
    _rng = _Rng(jax.random.key(int.from_bytes(__import__("os").urandom(4), "little")))
    _w = lambda a: (lambda t: t.astype(jnp.bfloat16) if jnp.issubdtype(t.dtype, jnp.floating) else t)(jnp.asarray(a))
    B, T, D, K = (2, 4000, 512, 15)
    return {'x': _w((lambda *s: _rng.normal(s) * 0.2)(B, T, D)), 'w_pw1': _w((lambda *s: _rng.normal(s) * 0.2)(D, 2 * D)), 'dw': _w((lambda *s: _rng.normal(s) * 0.05)(K, D)), 'w_pw2': _w((lambda *s: _rng.normal(s) * 0.05)(D, D))}

def reference(x, w_pw1, dw, w_pw2):
    B, T, D = x.shape
    K = dw.shape[0]
    h = x @ w_pw1
    a, b = (h[..., :D].copy(), h[..., D:].copy())
    h = a * _sigmoid(b)
    pad = K // 2
    hp = jnp.pad(h, ((0, 0), (pad, pad), (0, 0)))
    out = jnp.zeros_like(h)
    for i in range(K):
        out = out + hp[:, i:i + T, :] * dw[i][None, None, :]
    return _silu(out) @ w_pw2
```

```python
import functools
import jax
import jax.numpy as jnp
from jax import lax
import jax.experimental.pallas as pl
import jax.experimental.pallas.tpu as pltpu

F32 = jnp.float32
BF16 = jnp.bfloat16


def _sigmoid(v):
    return 0.5 * jnp.tanh(0.5 * v) + 0.5


def make(R=400, RS=16, G=16, U=2, unroll=False, flags=None, lead=0):
    def kern(x_hbm, w1_hbm, dw_hbm, w2_hbm, o_hbm, xv, w1_ref, dw_ref, w2_ref, h0, h1, y0, y1, ov, dwf, gsm, xsem, wsem, osem, *, N, T, D, K):
        NC = N // R
        CPB = T // R
        NL = D // 128
        pad = K // 2
        hb = (h0, h1)
        yb = (y0, y1)

        def x_copy(lo, n, slot):
            if not isinstance(lo, int):
                lo = pl.multiple_of(lo, 8)
            return pltpu.make_async_copy(x_hbm.at[pl.ds(lo, n)], xv.at[pl.ds(lo + 8, n)], xsem.at[slot])

        def o_copy(j):
            lo = j * R
            if not isinstance(lo, int):
                lo = pl.multiple_of(lo, 8)
            return pltpu.make_async_copy(ov.at[pl.ds(lo, R)], o_hbm.at[pl.ds(lo, R)], osem.at[0])

        def conv_piece(s, n, r):
            acc = None
            for i in range(K):
                t = hb[s][n, pl.ds(r + 8 - pad + i, RS), :] * jnp.tile(dwf[n, i], (RS // 8, 1))
                acc = t if acc is None else acc + t
            yv = acc * _sigmoid(acc)
            yb[s][r:r + RS, n * 128:(n + 1) * 128] = yv.astype(BF16)

        def run(passes, conv_slot, goff, ja=None, jc=None, sa=None, sc=None, first=False):
            pieces = [] if conv_slot is None else [(n, r) for n in range(NL) for r in range(0, R, RS)]
            ngates = sum(((R + 16) if (first and p != 'c') else R) // G for p, _ in passes)
            state = dict(g=0, done=0)

            def gate(v):
                state['g'] += 1
                if not pieces:
                    return
                want = min(len(pieces), (len(pieces) * (state['g'] + lead)) // ngates)
                if want > state['done']:
                    hb[conv_slot][pieces[state['done']][0], pl.ds(goff, 8), :] = v
                while state['done'] < want:
                    conv_piece(conv_slot, *pieces[state['done']])
                    state['done'] += 1

            def xrows():
                if first:
                    return xv[0:R + 16, :]
                lo = ja * R + 16
                if not isinstance(lo, int):
                    lo = pl.multiple_of(lo, 16)
                return xv[pl.ds(lo, R), :]

            a = None
            for p, n in passes:
                if p == 'a':
                    a = jnp.dot(xrows(), w1_ref[:, n * 128:(n + 1) * 128], preferred_element_type=F32)
                    for r in range(0, a.shape[0], G):
                        gate(a[r + G - 8:r + G])
                elif p == 'b':
                    b = jnp.dot(xrows(), w1_ref[:, D + n * 128:D + (n + 1) * 128], preferred_element_type=F32)
                    M = b.shape[0]
                    base = R + 16 - M
                    is_last = (ja % CPB) == (CPB - 1)
                    if first:
                        hb[sa][n, 0:8, :] = jnp.zeros((8, 128), F32)
                    else:
                        prev_last = (ja % CPB) == 0
                        hb[sa][n, 0:8, :] = jnp.where(prev_last, 0.0, hb[1 - sa][n, R:R + 8, :])
                        hb[sa][n, 8:16, :] = hb[1 - sa][n, R + 16:R + 24, :]
                    for r in range(0, M, G):
                        new = a[r:r + G] * _sigmoid(b[r:r + G])
                        lo = 8 if (first and r == 0) else 0
                        if r + G == M:
                            if G - 8 > lo:
                                hb[sa][n, base + r + lo:base + r + G - 8, :] = new[lo:G - 8]
                            hb[sa][n, R + 8:R + 16, :] = jnp.where(is_last, 0.0, new[G - 8:])
                            hb[sa][n, R + 16:R + 24, :] = new[G - 8:]
                        elif G > lo:
                            hb[sa][n, base + r + lo:base + r + G, :] = new[lo:]
                        gate(b[r + G - 8:r + G])
                else:
                    o = jnp.dot(yb[sc][...], w2_ref[:, n * 128:(n + 1) * 128], preferred_element_type=F32)
                    olo = jc * R
                    if not isinstance(olo, int):
                        olo = pl.multiple_of(olo, 16)
                    for r in range(0, R, G):
                        ov[pl.ds(olo + r, G), n * 128:(n + 1) * 128] = o[r:r + G].astype(BF16)
                        gate(o[r + G - 8:r + G])
            assert state['done'] == len(pieces)

        AB = [(p, n) for n in range(NL) for p in 'ab']
        ABC = [(p, n) for n in range(NL) for p in 'abc']
        C = [('c', n) for n in range(NL)]

        w1_copy = pltpu.make_async_copy(w1_hbm, w1_ref, wsem.at[0])
        dw_copy = pltpu.make_async_copy(dw_hbm, dw_ref, wsem.at[1])
        w2_copy = pltpu.make_async_copy(w2_hbm, w2_ref, wsem.at[2])
        c0 = x_copy(0, R + 8, 0)
        c1 = x_copy(R + 8, R, 1)
        w1_copy.start()
        c0.start()
        gsm[0] = R + 24
        xv[0:8, :] = jnp.zeros((8, D), BF16)
        xv[N + 8:N + 16, :] = jnp.zeros((8, D), BF16)
        w1_copy.wait()
        c0.wait()
        c1.start()
        dw_copy.start()
        w2_copy.start()
        run(AB, None, None, ja=0, sa=0, first=True)
        c1.wait()
        dw_copy.wait()
        NI = (NC - 2) // U
        assert NI * U == NC - 2 and U % 2 == 0

        def x_iter(p, last):
            return x_copy((U * p + 2) * R + 8, U * R - (8 if last else 0), p % 2)

        x_iter(0, NI == 1).start()
        for n in range(NL):
            for i in range(K):
                dwf[n, i] = jnp.broadcast_to(dw_ref[i:i + 1, n * 128:(n + 1) * 128].astype(F32), (8, 128))
        g0 = pl.multiple_of(gsm[0], 8)
        run(AB, 0, g0, ja=1, sa=1)
        w2_copy.wait()

        def body(p, _):
            if isinstance(p, int):
                x_iter(p, p == NI - 1).wait()
                if p + 1 < NI:
                    x_iter(p + 1, p + 1 == NI - 1).start()
            else:
                @pl.when(p < NI - 1)
                def _():
                    x_iter(p, False).wait()

                @pl.when(p == NI - 1)
                def _():
                    x_iter(p, True).wait()

                @pl.when(p + 1 < NI - 1)
                def _():
                    x_iter(p + 1, False).start()

                @pl.when(p + 1 == NI - 1)
                def _():
                    x_iter(p + 1, True).start()
            goff = pl.multiple_of(gsm[0], 8)
            for u in range(U):
                i = U * p + 1 + u
                s = (1 + u) % 2
                run(ABC, s, goff, ja=i + 1, jc=i - 1, sa=1 - s, sc=1 - s)
                o_copy(i - 1).start()
            return None

        if unroll:
            for p in range(NI):
                body(p, None)
        else:
            lax.fori_loop(0, NI, body, None)
        s = (NC - 1) % 2
        run(C, s, pl.multiple_of(gsm[0], 8), jc=NC - 2, sc=1 - s)
        o_copy(NC - 2).start()
        run(C, None, None, jc=NC - 1, sc=s)
        o_copy(NC - 1).start()
        pltpu.make_async_copy(ov, o_hbm, osem.at[0]).wait()

    @jax.jit
    def run(x, w_pw1, dw, w_pw2):
        B, T, D = x.shape
        K = dw.shape[0]
        N = B * T
        hbm = pl.BlockSpec(memory_space=pl.ANY)
        out = pl.pallas_call(
            functools.partial(kern, N=N, T=T, D=D, K=K),
            out_shape=jax.ShapeDtypeStruct((N, D), x.dtype),
            in_specs=[hbm] * 4,
            out_specs=hbm,
            scratch_shapes=[pltpu.VMEM((N + 16, D), BF16), pltpu.VMEM((D, 2 * D), BF16), pltpu.VMEM((K, D), BF16), pltpu.VMEM((D, D), BF16)]
            + [pltpu.VMEM((D // 128, R + 32, 128), F32)] * 2
            + [pltpu.VMEM((R, D), BF16)] * 2 + [pltpu.VMEM((N, D), BF16), pltpu.VMEM((D // 128, K, 8, 128), F32), pltpu.SMEM((1,), jnp.int32),
               pltpu.SemaphoreType.DMA((2,)), pltpu.SemaphoreType.DMA((3,)), pltpu.SemaphoreType.DMA((1,))],
            compiler_params=pltpu.CompilerParams(vmem_limit_bytes=64 * 1024 * 1024, flags=flags),
        )(x.reshape(N, D), w_pw1, dw, w_pw2)
        return out.reshape(B, T, D)

    return run


_impl = None


def pallas_standalone__conformer_conv_module__speech_kernel(x, w_pw1, dw, w_pw2):
    return make()(x, w_pw1, dw, w_pw2)
```

```python
import functools

import jax
import jax.numpy as jnp
from jax import lax
import jax.experimental.pallas as pl
import jax.experimental.pallas.tpu as pltpu

ROWS = 400
PIECE = 16
LANES = 128
HALO = 8


def _sigmoid(v):
    return 0.5 * jnp.tanh(0.5 * v) + 0.5


def _aligned(v, m):
    return v if isinstance(v, int) else pl.multiple_of(v, m)


def _lanes(n):
    return slice(n * LANES, (n + 1) * LANES)


def _kernel(x_hbm, w1_hbm, dw_hbm, w2_hbm, o_hbm,
            xv, wv, dwv, dwf, hs, y0, y1, ov, gate_row, sems, *, T):
    f32, bf16 = jnp.float32, jnp.bfloat16
    N, D = o_hbm.shape
    K = dw_hbm.shape[0]
    R, G = ROWS, PIECE
    NT = D // LANES
    NC = N // R
    CPB = T // R
    PT = R // G
    SP = 2 * PT // 5
    NI = (NC - 2) // 2
    ys = (y0, y1)

    def x_copy(lo, hi, sem):
        return pltpu.make_async_copy(
            x_hbm.at[lo:hi], xv.at[lo + HALO:hi + HALO], sems.at[sem])

    def w_copy(w_hbm, src, dst, sem):
        return pltpu.make_async_copy(w_hbm.at[:, _lanes(src)], wv.at[dst], sems.at[sem])

    def o_copy(lo, n, cols=slice(None)):
        lo = _aligned(lo, 8)
        return pltpu.make_async_copy(
            ov.at[pl.ds(lo, n), cols], o_hbm.at[pl.ds(lo, n), cols], sems.at[2])

    def conv_piece(slot, n, r):
        acc = None
        for i in range(K):
            t = hs[n, pl.ds(r + HALO - K // 2 + i, G), :] * jnp.tile(dwf[n, i], (G // 8, 1))
            acc = t if acc is None else acc + t
        ys[slot][n, r:r + G, :] = (acc * _sigmoid(acc)).astype(bf16)

    def pieces(slot, n, lo=0, hi=PT):
        return [(slot, n, q * G) for q in range(lo, hi)]

    def glu_passes(n, j):
        first = isinstance(j, int) and j == 0
        M = R + 16 if first else R
        rows = pl.ds(0 if first else _aligned(j * R + 16, 16), M)
        a = jnp.dot(xv[rows, :], wv[n], preferred_element_type=f32)
        for r in range(0, M, G):
            yield a[r + 8:r + G]
        b = jnp.dot(xv[rows, :], wv[NT + n], preferred_element_type=f32)
        if first:
            hs[n, 0:8, :] = jnp.zeros((8, LANES), f32)
        else:
            hs[n, 0:8, :] = jnp.where(j % CPB == 0, 0.0, hs[n, R:R + 8, :])
            hs[n, 8:16, :] = hs[n, R + 16:R + 24, :]
        base = R + 16 - M
        for r in range(0, M, G):
            h = a[r:r + G] * _sigmoid(b[r:r + G])
            if not (first and r == 0):
                hs[n, base + r:base + r + 8, :] = h[:8]
            if r + G < M:
                hs[n, base + r + 8:base + r + G, :] = h[8:]
            else:
                hs[n, R + 8:R + 16, :] = jnp.where(j % CPB == CPB - 1, 0.0, h[8:])
                hs[n, R + 16:R + 24, :] = h[8:]
            yield b[r + 8:r + G]

    def out_pass(n, j, slot, lo=0, hi=R, send_at=()):
        y = jnp.concatenate([ys[slot][k, lo:hi, :] for k in range(NT)], axis=1)
        o = jnp.dot(y, wv[2 * NT + n], preferred_element_type=f32)
        dst = ov.at[pl.ds(_aligned(j * R, 16), R)]
        sent = lo
        for r in range(lo, hi, G):
            dst[r:r + G, _lanes(n)] = o[r - lo:r - lo + G].astype(bf16)
            if r + G in send_at:
                o_copy(j * R + sent, r + G - sent, _lanes(n)).start()
                sent = r + G
            yield o[r - lo + 8:r - lo + G]

    def interleave(passes, todo=(), span=1):
        seen = done = 0
        for results in passes:
            for v in results:
                seen += 1
                want = min(len(todo), (len(todo) * seen + span - 1) // span)
                if want > done:
                    hs[0, pl.ds(gate, 8), :] = v
                while done < want:
                    conv_piece(*todo[done])
                    done += 1
        assert done == len(todo)

    def step(i, slot, resume=SP, drain=0):
        interleave([glu_passes(0, i + 1)], pieces(slot, NT - 1, resume), 2 * PT)
        for n in range(NT - 1):
            interleave([out_pass(n, i, slot), glu_passes(n + 1, i + 1)],
                       pieces(1 - slot, n), 3 * PT)
        interleave([out_pass(NT - 1, i, slot)], pieces(1 - slot, NT - 1, 0, SP), PT - drain)
        o_copy(i * R, R).start()

    groups = [range(0, 1), range(1, 2), range(2, NT)]
    loads = [[w_copy(w1_hbm, t, t, g) for n in tiles for t in (n, NT + n)]
             for g, tiles in enumerate(groups)]
    head = [pltpu.make_async_copy(dw_hbm, dwv, sems.at[0]), x_copy(0, R + HALO, 0)]
    w2_loads = [w_copy(w2_hbm, n, 2 * NT + n, 3) for n in range(NT)]
    x1_load = x_copy(R + HALO, 2 * R + HALO, 3)
    x_near = x_copy(2 * R + HALO, 6 * R + HALO, 0)
    x_far = x_copy(6 * R + HALO, N, 1)
    for c in head:
        c.start()

    @pl.loop(0, 2)
    def _(t):
        gate_row[t] = R + 24

    for c in sum(loads, []) + w2_loads:
        c.start()
    gate = pl.multiple_of(gate_row[0], 8)
    for g, tiles in enumerate(groups):
        for c in (head if g == 0 else []) + loads[g]:
            c.wait()
        if g == 0:
            xv[0:8, :] = jnp.zeros((8, D), bf16)
            xv[N + 8:N + 16, :] = jnp.zeros((8, D), bf16)
            x1_load.start()
            for n in range(NT):
                for i in range(K):
                    tap = dwv[i:i + 1, _lanes(n)].astype(f32)
                    dwf[n, i] = jnp.broadcast_to(tap, (8, LANES))
        for n in tiles:
            interleave([glu_passes(n, 0)], pieces(0, n - 1) if n else (),
                       2 * PT + (0 if n == tiles[-1] else 2))
    for c in w2_loads + [x1_load]:
        c.wait()
    x_near.start()
    x_far.start()
    step(0, 0, resume=0, drain=2)
    x_near.wait()

    def two_steps(p, carry):
        pl.when(p == 2)(x_far.wait)
        step(2 * p + 1, 1)
        step(2 * p + 2, 0, drain=2)
        return carry

    lax.fori_loop(0, NI, two_steps, None)

    j, M = NC - 1, SP * G
    interleave([out_pass(n, j, 1, 0, M) for n in range(NT)],
               pieces(1, NT - 1, SP), NT * SP - 12)
    o_copy(j * R, M).start()
    thirds = [M + (PT - SP) * q // 3 * G for q in (1, 2, 3)]
    interleave([out_pass(n, j, 1, M, R, thirds if n == NT - 1 else [R]) for n in range(NT)])
    pltpu.make_async_copy(ov, o_hbm, sems.at[2]).wait()


@jax.jit
def pallas_standalone__conformer_conv_module__speech_kernel(
    x: jax.Array,
    w_pw1: jax.Array,
    dw: jax.Array,
    w_pw2: jax.Array,
):
    B, T, D = x.shape
    K = dw.shape[0]
    N = B * T
    NT = D // LANES
    assert D == 4 * LANES and K // 2 <= HALO
    assert T % ROWS == 0 and (N // ROWS) % 2 == 0 and N // ROWS >= 8
    bf16, f32 = jnp.bfloat16, jnp.float32
    hbm = pl.BlockSpec(memory_space=pltpu.HBM)
    out = pl.pallas_call(
        functools.partial(_kernel, T=T),
        out_shape=jax.ShapeDtypeStruct((N, D), x.dtype),
        in_specs=[hbm] * 4,
        out_specs=hbm,
        scratch_shapes=[
            pltpu.VMEM((N + 2 * HALO, D), bf16),
            pltpu.VMEM((3 * NT, D, LANES), bf16),
            pltpu.VMEM((K, D), bf16),
            pltpu.VMEM((NT, K, 8, LANES), f32),
            pltpu.VMEM((NT, ROWS + 32, LANES), f32),
            pltpu.VMEM((NT, ROWS, LANES), bf16),
            pltpu.VMEM((NT, ROWS, LANES), bf16),
            pltpu.VMEM((N, D), bf16),
            pltpu.SMEM((2,), jnp.int32),
            pltpu.SemaphoreType.DMA((4,)),
        ],
        compiler_params=pltpu.CompilerParams(vmem_limit_bytes=48 * 1024 * 1024),
    )(x.reshape(N, D), w_pw1, dw, w_pw2)
    return out.reshape(B, T, D)
```
